```python
import jax
import jax.numpy as jnp

def _softmax(x, axis=-1):
    return jax.nn.softmax(x, axis=axis)
def _gelu(x):
    return jax.nn.gelu(x, approximate=True)
def _silu(x):
    return jax.nn.silu(x)
def _sigmoid(x):
    return jax.nn.sigmoid(x)
def _layernorm(x, axis=-1, eps=1e-5):
    m = jnp.mean(x, axis=axis, keepdims=True)
    v = jnp.var(x, axis=axis, keepdims=True)
    return (x - m) / jnp.sqrt(v + eps)
def _scatter_add(tgt, idx, src, axis=0):
    return tgt.at[idx].add(src)
def _segment_sum(src, seg, n):
    return jax.ops.segment_sum(src, seg, n)
class _Rng:
    def __init__(self, key):
        self._k = key
    def _next(self):
        self._k, sub = jax.random.split(self._k)
        return sub
    def normal(self, shape):
        return jax.random.normal(self._next(), shape, dtype=jnp.bfloat16)
    def randint(self, lo, hi, shape):
        return jax.random.randint(self._next(), shape, lo, hi, dtype=jnp.int32)
    def uniform(self, shape, lo=0.0, hi=1.0):
        return jax.random.uniform(self._next(), shape, jnp.bfloat16, lo, hi)
    def permutation(self, n):
        return jax.random.permutation(self._next(), n)


kernel_name = 'concat_heads__mha_block_cached__gqa_block_cached__near_ridge'

def _fwd_setup_inputs():
    _rng = _Rng(jax.random.key(int.from_bytes(__import__("os").urandom(4), "little")))
    _w = (lambda a: (lambda t: t.astype(jnp.bfloat16) if jnp.issubdtype(t.dtype, jnp.floating) else t)(jnp.asarray(a)))
    def _A_setup():
        B, Sq, D = 8, 224, 448
        H, Sk, Dh = 16, 512, 256
        return {
            "x": _w((lambda *s: _rng.normal(s) * 0.05)(B, Sq, D)),
            "k_cache": _w((lambda *s: _rng.normal(s) * 0.05)(B, H, Sk, Dh)),
            "v_cache": _w((lambda *s: _rng.normal(s) * 0.05)(B, H, Sk, Dh)),
            "wq": _w((lambda *s: _rng.normal(s) * 0.05)(D, H * Dh) * (D ** -0.5)),
            "wo": _w((lambda *s: _rng.normal(s) * 0.05)(H * Dh, D) * ((H * Dh) ** -0.5)),
        }
    _A_in = _A_setup()

    def _B_setup():
        B, Sq, D = 8, 224, 448
        Hq, Hkv, Sk, Dh = 16, 16, 512, 256
        assert Hq % Hkv == 0, (Hq, Hkv)
        return {
            "x": _w((lambda *s: _rng.normal(s) * 0.05)(B, Sq, D)),
            "k_cache": _w((lambda *s: _rng.normal(s) * 0.05)(B, Hkv, Sk, Dh)),
            "v_cache": _w((lambda *s: _rng.normal(s) * 0.05)(B, Hkv, Sk, Dh)),
            "wq": _w((lambda *s: _rng.normal(s) * 0.05)(D, Hq * Dh) * (D ** -0.5)),
            "wo": _w((lambda *s: _rng.normal(s) * 0.05)(Hq * Dh, D) * ((Hq * Dh) ** -0.5)),
        }
    _B_in = _B_setup()

    return {
        "A_x": _A_in["x"],
        "A_k_cache": _A_in["k_cache"],
        "A_v_cache": _A_in["v_cache"],
        "A_wq": _A_in["wq"],
        "A_wo": _A_in["wo"],
        "B_x": _B_in["x"],
        "B_k_cache": _B_in["k_cache"],
        "B_v_cache": _B_in["v_cache"],
        "B_wq": _B_in["wq"],
        "B_wo": _B_in["wo"],
    }

def _fwd_reference(A_x, A_k_cache, A_v_cache, A_wq, A_wo, B_x, B_k_cache, B_v_cache, B_wq, B_wo):
    def _A_ref(x, k_cache, v_cache, wq, wo):
        B, Sq, D = x.shape
        H, Dh = 16, 256
        q = (lambda x, *d: x.transpose(*d))((x @ wq).reshape(B, Sq, H, Dh), 0, 2, 1, 3)
        scores = jnp.einsum("bhqd,bhkd->bhqk", q, k_cache) * (Dh ** -0.5)
        p = _softmax(scores, axis=-1)
        o = jnp.einsum("bhqk,bhkd->bhqd", p, v_cache)
        return (lambda x, *d: x.transpose(*d))(o, 0, 2, 1, 3).reshape(B, Sq, H * Dh) @ wo

    def _B_ref(x, k_cache, v_cache, wq, wo):
        B, Sq, D = x.shape
        Hq, Dh = 16, 256
        Hkv = k_cache.shape[1]
        rep = Hq // Hkv
        q = (lambda x, *d: x.transpose(*d))((x @ wq).reshape(B, Sq, Hq, Dh), 0, 2, 1, 3)
        k = jnp.repeat(k_cache, rep, axis=1)
        v = jnp.repeat(v_cache, rep, axis=1)
        scores = jnp.einsum("bhqd,bhkd->bhqk", q, k) * (Dh ** -0.5)
        p = _softmax(scores, axis=-1)
        o = jnp.einsum("bhqk,bhkd->bhqd", p, v)
        return (lambda x, *d: x.transpose(*d))(o, 0, 2, 1, 3).reshape(B, Sq, Hq * Dh) @ wo

    a = _A_ref(A_x, A_k_cache, A_v_cache, A_wq, A_wo)
    b = _B_ref(B_x, B_k_cache, B_v_cache, B_wq, B_wo)
    return jnp.concatenate([a, b], axis=-1)


def setup_inputs():
    _inp = _fwd_setup_inputs()
    _gk = jax.random.fold_in(jax.random.key(int.from_bytes(__import__("os").urandom(4), "little")), 2**31 - 1)
    _shapes = [[8, 224, 896]]
    _dtypes = ['bfloat16']
    _gks = jax.random.split(_gk, len(_shapes))
    _gs = [jax.random.normal(k, s, dtype=jnp.dtype(d)) * 0.05 for k, s, d in zip(_gks, _shapes, _dtypes)]
    _inp["grad_out"] = _gs[0]
    return _inp

def reference(A_x, A_k_cache, A_v_cache, A_wq, A_wo, B_x, B_k_cache, B_v_cache, B_wq, B_wo, grad_out):
    _const = dict()
    def _f(*_d):
        return _fwd_reference(**{'A_x': _d[0], 'A_k_cache': _d[1], 'A_v_cache': _d[2], 'A_wq': _d[3], 'A_wo': _d[4], 'B_x': _d[5], 'B_k_cache': _d[6], 'B_v_cache': _d[7], 'B_wq': _d[8], 'B_wo': _d[9], **_const})
    _out, _vjp = jax.vjp(_f, A_x, A_k_cache, A_v_cache, A_wq, A_wo, B_x, B_k_cache, B_v_cache, B_wq, B_wo)
    _grads = _vjp(grad_out)
    _out0 = jnp.asarray(_out)
    return (_out0, *[jnp.asarray(_g) for _g in _grads])
```

```python
import jax
import jax.numpy as jnp
from jax import lax
import jax.experimental.pallas as pl
import jax.experimental.pallas.tpu as pltpu

CFG = dict(unroll=8, flags={})

B, SQ, D, H, SK, DH = 8, 224, 448, 16, 512, 256
M = B * SQ
SCALE = DH ** -0.5
BF, F32 = jnp.bfloat16, jnp.float32
NN = (((1,), (0,)), ((), ()))
NT = (((1,), (1,)), ((), ()))
TN = (((0,), (0,)), ((), ()))


def _dot(a, b, dims):
    return lax.dot_general(a, b, dims, preferred_element_type=F32)


def _kernel(xa, ka, va, wqa, woa, xb, kb, vb, wqb, wob, g_hbm,
            out_hbm, dxa, dka, dva, dwqa, dwoa, dxb, dkb, dvb, dwqb, dwob,
            x_s, g_raw, g_s, xt_s, gt_s, k_s, v_s, wq_s, wo_s, dk_s, dv_s, dwq_s, dwo_s,
            q_s, do_s, o_s, dq_s, outt_s, dxt_s, out_st, dx_st,
            sem_in, sem_w, sem_o, sem_p, sem_f):

    def in_copies(br, h, slot):
        k, v, wq, wo = ((ka, va, wqa, woa), (kb, vb, wqb, wob))[br]
        c0 = pl.multiple_of(h * DH, DH)
        return [
            pltpu.make_async_copy(wq.at[:, pl.ds(c0, DH)], wq_s.at[slot], sem_in.at[slot, 0]),
            pltpu.make_async_copy(wo.at[:, pl.ds(c0, DH)], wo_s.at[slot], sem_in.at[slot, 1]),
            pltpu.make_async_copy(k.at[:, h], k_s.at[slot], sem_in.at[slot, 2]),
            pltpu.make_async_copy(v.at[:, h], v_s.at[slot], sem_in.at[slot, 3]),
        ]

    def out_copies(br, h, slot):
        dk, dv, dwq, dwo = ((dka, dva, dwqa, dwoa), (dkb, dvb, dwqb, dwob))[br]
        c0 = pl.multiple_of(h * DH, DH)
        return [
            pltpu.make_async_copy(dk_s.at[slot], dk.at[:, h], sem_o.at[slot, 0]),
            pltpu.make_async_copy(dv_s.at[slot], dv.at[:, h], sem_o.at[slot, 1]),
            pltpu.make_async_copy(dwq_s.at[slot], dwq.at[:, pl.ds(c0, DH)], sem_o.at[slot, 2]),
            pltpu.make_async_copy(dwo_s.at[slot], dwo.at[:, pl.ds(c0, DH)], sem_o.at[slot, 3]),
        ]

    def for_step(t, fn):
        @pl.when(t < H)
        def _():
            fn(0, t)

        @pl.when(t >= H)
        def _():
            fn(1, t - H)

    cxa = pltpu.make_async_copy(xa, x_s.at[0], sem_p.at[0])
    cg = pltpu.make_async_copy(g_hbm, g_raw, sem_p.at[1])
    cxb = pltpu.make_async_copy(xb, x_s.at[1], sem_p.at[2])
    cxa.start()
    cg.start()
    for c in in_copies(0, 0, 0):
        c.start()
    cxb.start()
    cxa.wait()
    xt_s[0] = x_s[0].T
    cg.wait()
    g_s[0] = g_raw[:, :D]
    g_s[1] = g_raw[:, D:]
    gt = g_raw[...].T
    gt_s[0] = gt[:D]
    gt_s[1] = gt[D:]
    cxb.wait()
    xt_s[1] = x_s[1].T
    outt_s[...] = jnp.zeros(outt_s.shape, F32)
    dxt_s[...] = jnp.zeros(dxt_s.shape, F32)

    def step(t, carry):
        slot = t % 2
        br = t // H

        @pl.when(t + 1 < 2 * H)
        def _():
            for_step(t + 1, lambda b_, h_: [c.start() for c in in_copies(b_, h_, 1 - slot)])

        for c in in_copies(0, 0, slot):
            c.wait()

        @pl.when(t >= 2)
        def _():
            for c in out_copies(0, 0, slot):
                c.wait()

        wq = wq_s[slot] * jnp.asarray(SCALE, BF)
        wo = wo_s[slot]
        q_s[...] = _dot(x_s[br], wq, NN).astype(BF)
        do_s[...] = _dot(g_s[br], wo, NN).astype(BF)

        def attn(b):
            rows = pl.ds(b * SQ if isinstance(b, int) else pl.multiple_of(b * SQ, SQ), SQ)
            q = q_s[rows, :]
            do = do_s[rows, :]
            k = k_s[slot, b]
            v = v_s[slot, b]
            s = _dot(q, k, NT)
            dp = _dot(do, v, NT)
            m = jnp.max(s, axis=-1, keepdims=True)
            e = jnp.exp(s - m)
            l = jnp.sum(e, axis=-1, keepdims=True)
            p = e * (1.0 / l)
            pb = p.astype(BF)
            o_s[rows, :] = _dot(pb, v, NN).astype(BF)
            dv_s[slot, b] = _dot(pb, do, TN).astype(BF)
            delta = jnp.sum(p * dp, axis=-1, keepdims=True)
            ds = (p * (dp - delta)).astype(BF)
            dq_s[rows, :] = _dot(ds, k, NN).astype(BF)
            dk_s[slot, b] = _dot(ds, q, TN).astype(BF)

        U = CFG["unroll"]
        if U == B:
            for b in range(B):
                attn(b)
        else:
            def body(i, c):
                for u in range(U):
                    attn(i * U + u)
                return c
            lax.fori_loop(0, B // U, body, 0)

        outt_s[br] += _dot(wo, o_s[...], NT)
        dxt_s[br] += _dot(wq, dq_s[...], NT)
        dwq_s[slot] = (_dot(xt_s[br], dq_s[...], NN) * SCALE).astype(BF)
        dwo_s[slot] = _dot(gt_s[br], o_s[...], NN).astype(BF)
        for_step(t, lambda b_, h_: [c.start() for c in out_copies(b_, h_, slot)])
        return carry

    lax.fori_loop(0, 2 * H, step, 0)

    dx_st[0] = dxt_s[0].astype(BF).T
    c0 = pltpu.make_async_copy(dx_st.at[0], dxa, sem_f.at[0])
    c0.start()
    dx_st[1] = dxt_s[1].astype(BF).T
    c1 = pltpu.make_async_copy(dx_st.at[1], dxb, sem_f.at[1])
    c1.start()
    out_st[...] = outt_s[...].reshape(2 * D, M).astype(BF).T
    c2 = pltpu.make_async_copy(out_st, out_hbm, sem_f.at[2])
    c2.start()
    for slot in range(2):
        for c in out_copies(0, 0, slot):
            c.wait()
    c0.wait()
    c1.wait()
    c2.wait()


@jax.jit
def pallas_concat_heads__mha_block_cached__gqa_block_cached__near_ridge_kernel(
        A_x, A_k_cache, A_v_cache, A_wq, A_wo, B_x, B_k_cache, B_v_cache, B_wq, B_wo, grad_out):
    sds = jax.ShapeDtypeStruct
    branch = [sds((M, D), BF), sds((B, H, SK, DH), BF), sds((B, H, SK, DH), BF),
              sds((D, H * DH), BF), sds((D, H * DH), BF)]
    any_spec = pl.BlockSpec(memory_space=pltpu.HBM)
    vm = pltpu.VMEM
    outs = pl.pallas_call(
        _kernel,
        out_shape=[sds((M, 2 * D), BF)] + branch + branch,
        in_specs=[any_spec] * 11,
        out_specs=[any_spec] * 11,
        scratch_shapes=[
            vm((2, M, D), BF), vm((M, 2 * D), BF), vm((2, M, D), BF), vm((2, D, M), BF), vm((2, D, M), BF),
            vm((2, B, SK, DH), BF), vm((2, B, SK, DH), BF), vm((2, D, DH), BF), vm((2, D, DH), BF),
            vm((2, B, SK, DH), BF), vm((2, B, SK, DH), BF), vm((2, D, DH), BF), vm((2, D, DH), BF),
            vm((M, DH), BF), vm((M, DH), BF), vm((M, DH), BF), vm((M, DH), BF),
            vm((2, D, M), F32), vm((2, D, M), F32), vm((M, 2 * D), BF), vm((2, M, D), BF),
            pltpu.SemaphoreType.DMA((2, 4)), pltpu.SemaphoreType.DMA((2,)), pltpu.SemaphoreType.DMA((2, 4)),
            pltpu.SemaphoreType.DMA((3,)), pltpu.SemaphoreType.DMA((3,)),
        ],
        compiler_params=pltpu.CompilerParams(vmem_limit_bytes=110 * 1024 * 1024, flags=CFG["flags"] or None),
    )(A_x.reshape(M, D), A_k_cache, A_v_cache, A_wq, A_wo.T,
      B_x.reshape(M, D), B_k_cache, B_v_cache, B_wq, B_wo.T, grad_out.reshape(M, 2 * D))
    out, dxa, dka, dva, dwqa, dwoa, dxb, dkb, dvb, dwqb, dwob = outs
    return (out.reshape(B, SQ, 2 * D), dxa.reshape(B, SQ, D), dka, dva, dwqa, dwoa.T,
            dxb.reshape(B, SQ, D), dkb, dvb, dwqb, dwob.T)
```
